```python
import jax
import jax.numpy as jnp

def _softmax(x, axis=-1):
    return jax.nn.softmax(x, axis=axis)
def _gelu(x):
    return jax.nn.gelu(x, approximate=True)
def _silu(x):
    return jax.nn.silu(x)
def _sigmoid(x):
    return jax.nn.sigmoid(x)
def _layernorm(x, axis=-1, eps=1e-5):
    m = jnp.mean(x, axis=axis, keepdims=True)
    v = jnp.var(x, axis=axis, keepdims=True)
    return (x - m) / jnp.sqrt(v + eps)
def _scatter_add(tgt, idx, src, axis=0):
    return tgt.at[idx].add(src)
def _segment_sum(src, seg, n):
    return jax.ops.segment_sum(src, seg, n)
class _Rng:
    def __init__(self, key):
        self._k = key
    def _next(self):
        self._k, sub = jax.random.split(self._k)
        return sub
    def normal(self, shape):
        return jax.random.normal(self._next(), shape, dtype=jnp.bfloat16)
    def randint(self, lo, hi, shape):
        return jax.random.randint(self._next(), shape, lo, hi, dtype=jnp.int32)
    def uniform(self, shape, lo=0.0, hi=1.0):
        return jax.random.uniform(self._next(), shape, jnp.bfloat16, lo, hi)
    def permutation(self, n):
        return jax.random.permutation(self._next(), n)


kernel_name = 'interleave_layers__sliding_local_dilated__spectral_gfnet__prompt'

def setup_inputs():
    _rng = _Rng(jax.random.key(int.from_bytes(__import__("os").urandom(4), "little")))
    _w = (lambda a: (lambda t: t.astype(jnp.bfloat16) if jnp.issubdtype(t.dtype, jnp.floating) else t)(jnp.asarray(a)))
    def _A_setup():
        B, S, D = 1, 2048, 1024
        return {
            "x": _w((lambda *s: _rng.normal(s) * 0.05)(B, S, D)),
            "wqkv": _w((lambda *s: _rng.normal(s) * 0.05)(D, 3 * D)),
            "wo": _w((lambda *s: _rng.normal(s) * 0.05)(D, D)),
        }
    _A_in = _A_setup()

    def _B_setup():
        B, S, D = 1, 2048, 1024
        Df = D // 2 + 1
        return {
            "x": _w((lambda *s: _rng.normal(s) * 0.05)(B, S, D)),
            "w_r": _w((lambda *s: _rng.normal(s) * 0.05)(S, Df) * 0.02),
            "w_i": _w((lambda *s: _rng.normal(s) * 0.05)(S, Df) * 0.02),
        }
    _B_in = _B_setup()

    return {
        "A_x": _A_in["x"],
        "A_wqkv": _A_in["wqkv"],
        "A_wo": _A_in["wo"],
        "B_x": _B_in["x"],
        "B_w_r": _B_in["w_r"],
        "B_w_i": _B_in["w_i"],
    }

def reference(A_x, A_wqkv, A_wo, B_x, B_w_r, B_w_i):
    def _A_ref(x, wqkv, wo):
        B, S, D = x.shape
        H = 32; Dh = D // H
        W, dil = 8, 2
        qkv = (lambda x, *d: x.transpose(*d))((x @ wqkv).reshape(B, S, 3, H, Dh), 2, 0, 3, 1, 4)
        q, k, v = qkv[0], qkv[1], qkv[2]
        scale = Dh ** -0.5
        pos = jnp.arange(S)
        off = jnp.arange(W) * dil
        idx = pos[:, None] - off[None, :]
        mask = idx >= 0
        idx_c = jnp.where(mask, idx, 0).reshape(-1)
        kg = k[:, :, idx_c, :].reshape(B, H, S, W, Dh)
        vg = v[:, :, idx_c, :].reshape(B, H, S, W, Dh)
        logits = jnp.einsum("bhsd,bhswd->bhsw", q, kg) * scale
        logits = jnp.where(mask[None, None, :, :], logits, -1e9)
        attn = _softmax(logits, axis=-1)
        o = jnp.einsum("bhsw,bhswd->bhsd", attn, vg)
        return (lambda x, *d: x.transpose(*d))(o, 0, 2, 1, 3).reshape(B, S, D) @ wo

    def _B_ref(x, w_r, w_i):
        B, S, D = x.shape
        X = (lambda x, axes=(-2,-1): jnp.fft.rfft2(x.astype(jnp.float32), axes=axes))(x, axes=(-2, -1))
        W = w_r + 1j * w_i
        X = X * W
        y = (lambda x, s, axes=(-2,-1): jnp.fft.irfft2(x, s=s, axes=axes).astype(jnp.bfloat16))(X, (S, D), axes=(-2, -1))
        return y

    x = A_x
    x = x + _A_ref(_layernorm(x, axis=-1), A_wqkv, A_wo)
    x = x + _B_ref(_layernorm(x, axis=-1), B_w_r, B_w_i)
    x = x + _A_ref(_layernorm(x, axis=-1), A_wqkv, A_wo)
    x = x + _B_ref(_layernorm(x, axis=-1), B_w_r, B_w_i)
    return x
```

```python
import numpy as np
import jax
import jax.numpy as jnp
from jax import lax
import jax.experimental.pallas as pl
import jax.experimental.pallas.tpu as pltpu

S, D, H, DH, WIN = 2048, 1024, 32, 32, 8
NS, L = 16, 128
FR = 528
F32, BF16 = jnp.float32, jnp.bfloat16
NT = (((1,), (1,)), ((), ()))


def _consts():
    i = np.arange(L)
    hs = []
    for n1 in range(NS):
        h = np.exp(-2j * np.pi * np.outer(n1 + NS * i, i) / S)
        hs.append(np.block([[h.real, h.imag], [-h.imag, h.real]]))

    def e(r):
        return np.exp(-2j * np.pi * np.outer(r + 8 * np.arange(64), i) / D)

    ny = np.zeros((16, L))
    ny[0] = np.cos(np.pi * i)
    g0 = np.concatenate([e(0).real, e(0).imag, ny])
    g4 = np.concatenate([e(4).real, e(4).imag])
    gc = []
    for r, sg in ((1, -1.0), (2, -1.0), (3, 1.0)):
        a, b = e(r), e(8 - r)
        gc.append(np.block([[a.real, -sg * a.imag], [b.real, sg * b.imag],
                            [a.imag, sg * a.real], [b.imag, -sg * b.real]]))
    gc = np.stack(gc)
    out = (np.stack(hs), g0, g4, gc, g0.T, g4.T, gc.transpose(0, 2, 1))
    return tuple(np.ascontiguousarray(o).astype(BF16) for o in out)


_CONSTS = _consts()


def _cmul(xr, xi, k, n):
    c, s = np.cos(2 * np.pi * k / n), np.sin(2 * np.pi * k / n)
    if abs(abs(c) - abs(s)) < 1e-12:
        c = np.float32(c)
        if c * s > 0:
            return (xr - xi) * c, (xr + xi) * c
        return (xr + xi) * c, (xi - xr) * c
    c, s = np.float32(c), np.float32(s)
    return xr * c - xi * s, xr * s + xi * c


def _fft(x, sg):
    n = len(x)
    if n == 1:
        return x
    ev, od = _fft(x[0::2], sg), _fft(x[1::2], sg)
    lo, hi = [], []
    for k in range(n // 2):
        (er, ei), (tr, ti) = ev[k], od[k]
        if 4 * k == n:
            p, m = (er - ti, ei + tr), (er + ti, ei - tr)
            p, m = (p, m) if sg > 0 else (m, p)
        else:
            if k:
                tr, ti = _cmul(tr, ti, sg * k, n)
            p, m = (er + tr, ei + ti), (er - tr, ei - ti)
        lo.append(p)
        hi.append(m)
    return lo + hi


def _dot(a, b):
    return jnp.dot(a, b, preferred_element_type=F32)


def _layernorm(x):
    m = jnp.sum(x, axis=0, keepdims=True) * (1.0 / D)
    c = x - m
    v = jnp.sum(c * c, axis=0, keepdims=True) * (1.0 / D)
    return c * lax.rsqrt(v + 1e-5)


def _kernel(x_hbm, wqkv_hbm, wo_hbm, wr_hbm, wi_hbm, hs_hbm, g0, g4, gc, a0, a4, ac,
            out_hbm, xt, xb, wraw, wt, fraw, filt, hs, q, kv, ot, yf, yb, sems):
    cp_x = pltpu.make_async_copy(x_hbm, xb, sems.at[0])
    cp_wqkv = pltpu.make_async_copy(wqkv_hbm, wraw.at[:, pl.ds(0, 3 * D)], sems.at[1])
    cp_wo = pltpu.make_async_copy(wo_hbm, wraw.at[:, pl.ds(3 * D, D)], sems.at[2])
    cp_wr = pltpu.make_async_copy(wr_hbm, fraw.at[0], sems.at[3])
    cp_wi = pltpu.make_async_copy(wi_hbm, fraw.at[1], sems.at[4])
    cp_hs = pltpu.make_async_copy(hs_hbm, hs, sems.at[5])
    for c in (cp_x, cp_wqkv, cp_wo, cp_wr, cp_wi, cp_hs):
        c.start()

    cp_x.wait()
    with jax.named_scope("prep_x"):
        @pl.loop(0, S // 64)
        def _(i):
            r = pl.ds(pl.multiple_of(i * 64, 64), 64)
            for c in range(8):
                kv[c, r, :] = xb[r, c * L:(c + 1) * L].astype(F32)

        @pl.loop(0, NS)
        def _(n1):
            for c in range(8):
                xt[n1, c * L:(c + 1) * L, :] = kv[c, pl.ds(n1, L, stride=NS), :].T

    cp_wqkv.wait()
    cp_wo.wait()
    with jax.named_scope("prep_w"):
        for c in range(4 * D // L):
            wt[c * L:(c + 1) * L, :] = wraw[:, c * L:(c + 1) * L].T

    cp_wr.wait()
    cp_wi.wait()
    with jax.named_scope("prep_f"):
        row = lax.broadcasted_iota(jnp.int32, (64, L), 0)
        sc = np.float32(2.0 / (S * D))
        sc0 = jnp.where(row == 0, sc * 0.5, sc)
        row16 = lax.broadcasted_iota(jnp.int32, (16, L), 0)

        @pl.loop(0, 2)
        def _(p):
            for k1 in range(NS):
                j, cs = p * NS + k1, slice(k1 * L, (k1 + 1) * L)
                kv[k1, 0:512, :] = fraw[p, 0:512, cs].astype(F32)
                for b in range(8):
                    filt[j, b * 64:(b + 1) * 64, :] = (
                        kv[k1, pl.ds(b, 64, stride=8), :] * (sc0 if b == 0 else sc))
                ny = jnp.broadcast_to(fraw[p, 512:513, cs].astype(F32), (16, L))
                filt[j, 512:FR, :] = jnp.where(row16 == 0, ny * (sc * 0.5), 0.0)

    cp_hs.wait()
    lane = lax.broadcasted_iota(jnp.int32, (8, L), 1)
    cc = np.float32(np.sqrt(0.5))

    @pl.loop(0, 2)
    def _(layer):
        with jax.named_scope("qkv"):
            @pl.loop(0, NS)
            def _(n1):
                xn = _layernorm(xt[n1]).astype(BF16)
                q[n1] = _dot(wt[0:D, :], xn) * np.float32(DH ** -0.5)
                for b in range(2):
                    t = _dot(wt[(b + 1) * D:(b + 2) * D, :], xn)
                    kv[NS + n1, b * D:(b + 1) * D, :] = t
                    kv[n1, b * D:(b + 1) * D, :] = pltpu.roll(t, 1, 1)

        with jax.named_scope("attn"):
            @pl.loop(0, NS)
            def _(n1):
                @pl.loop(0, H // 4)
                def _(g):
                    for hh in range(4):
                        r0 = pl.multiple_of(g * L + hh * DH, DH)
                        qh = q[n1, pl.ds(r0, DH), :]
                        lg = []
                        for w in range(WIN):
                            p = qh * kv[NS + n1 - 2 * w, pl.ds(r0, DH), :]
                            p = (p[0:8] + p[8:16]) + (p[16:24] + p[24:32])
                            for sh in (4, 2, 1):
                                p = p + pltpu.roll(p, sh, 0)
                            if w:
                                p = jnp.where((lane > 0) | (n1 >= 2 * w), p, -1e9)
                            lg.append(p)
                        mx = lg[0]
                        for p in lg[1:]:
                            mx = jnp.maximum(mx, p)
                        ex = [jnp.exp(p - mx) for p in lg]
                        sm = ex[0]
                        for p in ex[1:]:
                            sm = sm + p
                        inv = 1.0 / sm
                        o = None
                        for w in range(WIN):
                            v = kv[NS + n1 - 2 * w, pl.ds(D + r0, DH), :].reshape(4, 8, L)
                            t = v * ex[w][None]
                            o = t if o is None else o + t
                        o = (o * inv[None]).reshape(DH, L)
                        ot[n1, pl.ds(r0, DH), :] = o.astype(BF16)

        with jax.named_scope("proj_fwd"):
            @pl.loop(0, NS)
            def _(n1):
                x = xt[n1] + _dot(wt[3 * D:4 * D, :], ot[n1])
                xt[n1] = x
                xn = _layernorm(x)
                xs = [xn[j * L:(j + 1) * L] for j in range(8)]
                a = [xs[j] + xs[j + 4] for j in range(4)]
                b = [xs[j] - xs[j + 4] for j in range(4)]
                ev, od = a[0] + a[2], a[1] + a[3]
                t1, t2 = (b[1] - b[3]) * cc, (b[1] + b[3]) * cc
                z0 = _dot(g0[...], (ev + od).astype(BF16)).astype(BF16)
                z4 = _dot(g4[...], (ev - od).astype(BF16)).astype(BF16)
                zc = []
                for k, (ur, ui) in enumerate(((b[0] + t1, b[2] + t2),
                                              (a[0] - a[2], a[1] - a[3]),
                                              (b[0] - t1, b[2] - t2))):
                    u = jnp.concatenate([ur.astype(BF16), ui.astype(BF16)], axis=0)
                    zc.append(_dot(gc[k], u).astype(BF16))
                parts = []
                for o in (0, 1):
                    parts.append(jnp.concatenate(
                        [z0[o * 64:o * 64 + 64]]
                        + [zc[k][o * L:o * L + 64] for k in range(3)]
                        + [z4[o * 64:o * 64 + 64]]
                        + [zc[k][o * L + 64:o * L + L] for k in (2, 1, 0)]
                        + [z0[L:L + 16] if o == 0 else jnp.zeros((16, L), BF16)], axis=0))
                yf[n1] = _dot(jnp.concatenate(parts, axis=1), hs[n1])

        with jax.named_scope("mid"):
            @pl.loop(0, FR // 16)
            def _(i):
                res = []
                for hf in range(2):
                    r = pl.ds(pl.multiple_of(i * 16 + hf * 8, 8), 8)
                    z = _fft([(yf[j, r, 0:L], yf[j, r, L:2 * L]) for j in range(NS)], -1)
                    u = []
                    for j, (zr, zi) in enumerate(z):
                        fr, fi = filt[j, r, :], filt[NS + j, r, :]
                        u.append((zr * fr - zi * fi, zr * fi + zi * fr))
                    res.append(_fft(u, 1))
                r = pl.ds(pl.multiple_of(i * 16, 16), 16)
                for j in range(NS):
                    for o in range(2):
                        yb[j, r, o * L:(o + 1) * L] = jnp.concatenate(
                            [res[0][j][o], res[1][j][o]], axis=0).astype(BF16)

        with jax.named_scope("inv"):
            @pl.loop(0, NS)
            def _(n1):
                z = lax.dot_general(yb[n1], hs[n1], NT, preferred_element_type=F32).astype(BF16)
                blk = lambda r, o: z[r * 64:r * 64 + 64, o * L:(o + 1) * L]
                v0 = _dot(a0[...], jnp.concatenate(
                    [blk(0, 0), blk(0, 1), z[512:FR, 0:L]], axis=0))
                v4 = _dot(a4[...], jnp.concatenate([blk(4, 0), blk(4, 1)], axis=0))
                vc = [_dot(ac[k], jnp.concatenate(
                    [blk(k + 1, 0), blk(7 - k, 0), blk(k + 1, 1), blk(7 - k, 1)], axis=0))
                    for k in range(3)]
                (v1r, v1i), (v2r, v2i), (v3r, v3i) = [(v[0:L], v[L:2 * L]) for v in vc]
                ev, od = v0 + v4, v0 - v4
                a = [ev + v2r, od + v2i, ev - v2r, od - v2i]
                t1, t2 = v1r - v3r, v1i - v3i
                b = [v1r + v3r, (t1 + t2) * cc, v1i + v3i, (t2 - t1) * cc]
                for j in range(4):
                    xt[n1, j * L:(j + 1) * L, :] += a[j] + b[j]
                    xt[n1, (j + 4) * L:(j + 5) * L, :] += a[j] - b[j]

    with jax.named_scope("out"):
        @pl.loop(0, NS)
        def _(n1):
            for c in range(8):
                kv[c, pl.ds(n1, L, stride=NS), :] = xt[n1, c * L:(c + 1) * L, :].T

        @pl.loop(0, S // 64)
        def _(i):
            r = pl.ds(pl.multiple_of(i * 64, 64), 64)
            for c in range(8):
                xb[r, c * L:(c + 1) * L] = kv[c, r, :].astype(BF16)

    cp_o = pltpu.make_async_copy(xb, out_hbm, sems.at[0])
    cp_o.start()
    cp_o.wait()


@jax.jit
def pallas_interleave_layers__sliding_local_dilated__spectral_gfnet__prompt_kernel(
        A_x, A_wqkv, A_wo, B_x, B_w_r, B_w_i):
    del B_x
    hbm = pl.BlockSpec(memory_space=pltpu.HBM)
    vmem = pl.BlockSpec(memory_space=pltpu.VMEM)
    out = pl.pallas_call(
        _kernel,
        out_shape=jax.ShapeDtypeStruct((S, D), BF16),
        in_specs=[hbm] * 6 + [vmem] * 6,
        out_specs=hbm,
        scratch_shapes=[
            pltpu.VMEM((NS, D, L), F32),
            pltpu.VMEM((S, D), BF16),
            pltpu.VMEM((D, 4 * D), BF16),
            pltpu.VMEM((4 * D, D), BF16),
            pltpu.VMEM((2, D // 2 + 1, S), BF16),
            pltpu.VMEM((2 * NS, FR, L), F32),
            pltpu.VMEM((NS, 2 * L, 2 * L), BF16),
            pltpu.VMEM((NS, D, L), F32),
            pltpu.VMEM((2 * NS, 2 * D, L), F32),
            pltpu.VMEM((NS, D, L), BF16),
            pltpu.VMEM((NS, FR, 2 * L), F32),
            pltpu.VMEM((NS, FR, 2 * L), BF16),
            pltpu.SemaphoreType.DMA((6,)),
        ],
        compiler_params=pltpu.CompilerParams(vmem_limit_bytes=124 * 1024 * 1024),
    )(A_x.reshape(S, D), A_wqkv, A_wo, B_w_r.T, B_w_i.T, *_CONSTS)
    return out.reshape(1, S, D)
```

```python
import numpy as np
import jax
import jax.numpy as jnp
from jax import lax
import jax.experimental.pallas as pl
import jax.experimental.pallas.tpu as pltpu

S, D, H, DH, WIN = 2048, 1024, 32, 32, 8
NS, L = 16, 128
FR = 528
F32, BF16 = jnp.float32, jnp.bfloat16
NT = (((1,), (1,)), ((), ()))


def _consts():
    i = np.arange(L)
    hs = []
    for n1 in range(NS):
        h = np.exp(-2j * np.pi * np.outer(n1 + NS * i, i) / S)
        hs.append(np.block([[h.real, h.imag], [-h.imag, h.real]]))

    def e(r):
        return np.exp(-2j * np.pi * np.outer(r + 8 * np.arange(64), i) / D)

    ny = np.zeros((16, L))
    ny[0] = np.cos(np.pi * i)
    g0 = np.concatenate([e(0).real, e(0).imag, ny])
    g4 = np.concatenate([e(4).real, e(4).imag])
    gc = []
    for r, sg in ((1, -1.0), (2, -1.0), (3, 1.0)):
        a, b = e(r), e(8 - r)
        gc.append(np.block([[a.real, -sg * a.imag], [b.real, sg * b.imag],
                            [a.imag, sg * a.real], [b.imag, -sg * b.real]]))
    gc = np.stack(gc)
    out = (np.stack(hs), g0, g4, gc, g0.T, g4.T, gc.transpose(0, 2, 1))
    return tuple(np.ascontiguousarray(o).astype(BF16) for o in out)


_CONSTS = _consts()


def _cmul(xr, xi, k, n):
    c, s = np.cos(2 * np.pi * k / n), np.sin(2 * np.pi * k / n)
    if abs(abs(c) - abs(s)) < 1e-12:
        c = np.float32(c)
        if c * s > 0:
            return (xr - xi) * c, (xr + xi) * c
        return (xr + xi) * c, (xi - xr) * c
    c, s = np.float32(c), np.float32(s)
    return xr * c - xi * s, xr * s + xi * c


def _fft(x, sg):
    n = len(x)
    if n == 1:
        return x
    ev, od = _fft(x[0::2], sg), _fft(x[1::2], sg)
    lo, hi = [], []
    for k in range(n // 2):
        (er, ei), (tr, ti) = ev[k], od[k]
        if 4 * k == n:
            p, m = (er - ti, ei + tr), (er + ti, ei - tr)
            p, m = (p, m) if sg > 0 else (m, p)
        else:
            if k:
                tr, ti = _cmul(tr, ti, sg * k, n)
            p, m = (er + tr, ei + ti), (er - tr, ei - ti)
        lo.append(p)
        hi.append(m)
    return lo + hi


def _dot(a, b):
    return jnp.dot(a, b, preferred_element_type=F32)


def _layernorm(x):
    m = jnp.sum(x, axis=0, keepdims=True) * (1.0 / D)
    c = x - m
    v = jnp.sum(c * c, axis=0, keepdims=True) * (1.0 / D)
    return c * lax.rsqrt(v + 1e-5)


def _interleave(*gens):
    gens = list(gens)
    while gens:
        gens = [g for g in gens if next(g, 0) is None]


def _kernel(x_hbm, wqkv_hbm, wo_hbm, wr_hbm, wi_hbm, hs_hbm, g0, g4, gc, a0, a4, ac,
            out_hbm, xt, xb, wraw, wt, fraw, fst, filt, hs, xn, q, kv, ot, yf, yb, sems):
    col = lambda c, n=L: pl.ds(c * n, n)
    cp_w = [pltpu.make_async_copy(wqkv_hbm.at[:, col(c, D)], wraw.at[c], sems.at[c])
            for c in range(3)]
    cp_w.append(pltpu.make_async_copy(wo_hbm, wraw.at[3], sems.at[3]))
    cp_r = [pltpu.make_async_copy(wr_hbm, fraw.at[0], sems.at[4]),
            pltpu.make_async_copy(wi_hbm, fraw.at[1], sems.at[5]),
            pltpu.make_async_copy(hs_hbm, hs, sems.at[6])]
    cp_x = [pltpu.make_async_copy(x_hbm.at[:, col(c)], xb.at[c], sems.at[8 + c])
            for c in range(8)]
    for c in cp_w[1:3] + cp_x:
        c.start()
    xw = xb.bitcast(jnp.int32)

    with jax.named_scope("prep"):
        for b in (1, 2):
            cp_w[b].wait()
            for c in range(8):
                wt[col(8 * b + c), :] = wraw[b, :, col(c)].T
        for c in range(8):
            cp_x[c].wait()
            if c == 5:
                for d in [cp_w[0], cp_w[3]] + cp_r:
                    d.start()
            for j in range(NS // 2):
                w = xw[c, pl.ds(j, L, stride=NS // 2), :].T
                xt[2 * j, col(c), :] = lax.bitcast_convert_type(w << 16, F32)
                xt[2 * j + 1, col(c), :] = lax.bitcast_convert_type(w & -65536, F32)

    lane = lax.broadcasted_iota(jnp.int32, (8, L), 1)
    cc = np.float32(np.sqrt(0.5))
    CH = 4
    RC = D // CH

    def prep_rest(t):
        o = pl.ds(pl.multiple_of(t * L, L), L)
        for b in (0, 3):
            wt[pl.ds(pl.multiple_of(b * D + t * L, L), L), :] = wraw[b, :, o].T
            yield
        sc = np.float32(2.0 / (S * D))
        sc0 = jnp.where(lax.broadcasted_iota(jnp.int32, (64, L), 0) == 0, sc * 0.5, sc)
        row16 = lax.broadcasted_iota(jnp.int32, (16, L), 0)
        for p in range(2):
            for e in range(2):
                k1 = 2 * t + e
                cs = pl.ds(pl.multiple_of(k1 * L, L), L)
                fst[2 * p + e] = fraw[p, 0:512, cs].astype(F32)
                for b in range(8):
                    filt[p * NS + k1, col(b, 64), :] = (
                        fst[2 * p + e, pl.ds(b, 64, stride=8), :] * (sc0 if b == 0 else sc))
                ny = jnp.broadcast_to(fraw[p, 512:513, cs].astype(F32), (16, L))
                filt[p * NS + k1, 512:FR, :] = jnp.where(row16 == 0, ny * (sc * 0.5), 0.0)
                yield

    def ln_in(n1):
        yield
        xn[n1] = _layernorm(xt[n1]).astype(BF16)

    def kv_proj(n1):
        xv = xn[n1]
        for c in range(2 * CH):
            t = _dot(wt[pl.ds(D + c * RC, RC), :], xv)
            kv[NS + n1, col(c, RC), :] = t
            kv[n1, col(c, RC), :] = pltpu.roll(t, 1, 1)
            yield

    def q_proj(n1):
        xv = xn[n1]
        for c in range(CH):
            yield
            q[col(c, RC), :] = _dot(wt[col(c, RC), :], xv) * np.float32(DH ** -0.5)
            yield

    def attn(n1):
        for h in range(H):
            r = col(h, DH)
            qh = q[r, :]
            lg = []
            for w in range(WIN):
                p = qh * kv[NS + n1 - 2 * w, r, :]
                p = (p[0:8] + p[8:16]) + (p[16:24] + p[24:32])
                for sh in (4, 2, 1):
                    p = p + pltpu.roll(p, sh, 0)
                if w:
                    p = jnp.where((lane > 0) | (n1 >= 2 * w), p, -1e9)
                lg.append(p)
            mx = lg[0]
            for p in lg[1:]:
                mx = jnp.maximum(mx, p)
            ex = [jnp.exp(p - mx) for p in lg]
            sm = ex[0]
            for p in ex[1:]:
                sm = sm + p
            inv = 1.0 / sm
            o = None
            for w in range(WIN):
                t = kv[NS + n1 - 2 * w, col(H + h, DH), :].reshape(4, 8, L) * ex[w][None]
                o = t if o is None else o + t
            ot[n1, r, :] = (o * inv[None]).reshape(DH, L).astype(BF16)
            if h % 4 == 3:
                yield

    def out_proj(n1):
        ov = ot[n1]
        for c in range(CH):
            xt[n1, col(c, RC), :] += _dot(wt[pl.ds(3 * D + c * RC, RC), :], ov)
            yield
            yield

    def fwd(n1):
        x = _layernorm(xt[n1])
        yield
        xs = [x[j * L:(j + 1) * L] for j in range(8)]
        a = [xs[j] + xs[j + 4] for j in range(4)]
        b = [xs[j] - xs[j + 4] for j in range(4)]
        ev, od = a[0] + a[2], a[1] + a[3]
        t1, t2 = (b[1] - b[3]) * cc, (b[1] + b[3]) * cc
        yield
        z0 = _dot(g0[...], (ev + od).astype(BF16)).astype(BF16)
        z4 = _dot(g4[...], (ev - od).astype(BF16)).astype(BF16)
        zc = []
        for k, (ur, ui) in enumerate(((b[0] + t1, b[2] + t2), (a[0] - a[2], a[1] - a[3]),
                                      (b[0] - t1, b[2] - t2))):
            yield
            u = jnp.concatenate([ur.astype(BF16), ui.astype(BF16)], axis=0)
            zc.append(_dot(gc[k], u).astype(BF16))
        parts = []
        for o in (0, 1):
            parts.append(jnp.concatenate(
                [z0[o * 64:o * 64 + 64]] + [zc[k][o * L:o * L + 64] for k in range(3)]
                + [z4[o * 64:o * 64 + 64]] + [zc[k][o * L + 64:o * L + L] for k in (2, 1, 0)]
                + [z0[L:L + 16] if o == 0 else jnp.zeros((16, L), BF16)], axis=0))
        yield
        yf[n1] = _dot(jnp.concatenate(parts, axis=1), hs[n1])

    def mid(i):
        res = []
        for hf in range(2):
            r = pl.ds(pl.multiple_of(i * 16 + hf * 8, 8), 8)
            z = _fft([(yf[j, r, 0:L], yf[j, r, L:2 * L]) for j in range(NS)], -1)
            u = []
            for j, (zr, zi) in enumerate(z):
                fr, fi = filt[j, r, :], filt[NS + j, r, :]
                u.append((zr * fr - zi * fi, zr * fi + zi * fr))
            res.append(_fft(u, 1))
        r = pl.ds(pl.multiple_of(i * 16, 16), 16)
        for j in range(NS):
            for o in range(2):
                yb[j, r, col(o)] = jnp.concatenate(
                    [res[0][j][o], res[1][j][o]], axis=0).astype(BF16)

    def inv(n1):
        z = lax.dot_general(yb[n1], hs[n1], NT, preferred_element_type=F32).astype(BF16)
        blk = lambda r, o: z[r * 64:r * 64 + 64, o * L:(o + 1) * L]
        yield
        v0 = _dot(a0[...], jnp.concatenate([blk(0, 0), blk(0, 1), z[512:FR, 0:L]], axis=0))
        v4 = _dot(a4[...], jnp.concatenate([blk(4, 0), blk(4, 1)], axis=0))
        vc = []
        for k in range(3):
            yield
            vc.append(_dot(ac[k], jnp.concatenate(
                [blk(k + 1, 0), blk(7 - k, 0), blk(k + 1, 1), blk(7 - k, 1)], axis=0)))
        yield
        (v1r, v1i), (v2r, v2i), (v3r, v3i) = [(v[0:L], v[L:2 * L]) for v in vc]
        ev, od = v0 + v4, v0 - v4
        a = [ev + v2r, od + v2i, ev - v2r, od - v2i]
        t1, t2 = v1r - v3r, v1i - v3i
        b = [v1r + v3r, (t1 + t2) * cc, v1i + v3i, (t2 - t1) * cc]
        for j in range(4):
            xt[n1, col(j), :] += a[j] + b[j]
            xt[n1, col(j + 4), :] += a[j] - b[j]

    def pipeline(name, stages, cuts=()):
        end = max(g + n for _, g, n in stages)
        pts = sorted({0, end, *cuts, *[g for _, g, _ in stages], *[g + n for _, g, n in stages]})
        with jax.named_scope(name):
            for lo, hi in zip(pts, pts[1:]):
                if lo in cuts:
                    for d in [cp_w[0], cp_w[3]] + cp_r:
                        d.wait()

                def body(t, lo=lo):
                    _interleave(*[fn(t - g) for fn, g, n in stages if g <= lo < g + n])
                if hi - lo == 1:
                    body(lo)
                else:
                    pl.loop(lo, hi)(body)

    for layer in range(2):
        if layer == 0:
            pipeline("kv0", [(kv_proj, 1, NS), (ln_in, 0, NS), (prep_rest, 7, 8),
                             (q_proj, NS, 1)], cuts=(7,))
        else:
            pipeline("kv1", [(kv_proj, 2, NS), (ln_in, 1, NS), (inv, 0, NS), (q_proj, NS + 1, 1)])
        pipeline("att", [(fwd, 2, NS), (out_proj, 1, NS), (attn, 0, NS),
                         (lambda t: q_proj(t + 1), 0, NS - 1)])
        with jax.named_scope("mid"):
            pl.loop(0, FR // 16)(mid)
    with jax.named_scope("inv"):
        pl.loop(0, NS // 2)(lambda t: _interleave(inv(2 * t), inv(2 * t + 1)))

    with jax.named_scope("out"):
        cp_o = [pltpu.make_async_copy(xb.at[c], out_hbm.at[:, col(c)], sems.at[8 + c])
                for c in range(8)]
        bits = lambda v: lax.bitcast_convert_type(v.astype(BF16).astype(F32), jnp.int32)
        for c in range(8):
            for j in range(NS // 2):
                w = (lax.shift_right_logical(bits(xt[2 * j, col(c), :]), 16)
                     | bits(xt[2 * j + 1, col(c), :]))
                xw[c, pl.ds(j, L, stride=NS // 2), :] = w.T
            cp_o[c].start()
        for d in cp_o:
            d.wait()


@jax.jit
def pallas_interleave_layers__sliding_local_dilated__spectral_gfnet__prompt_kernel(
        A_x, A_wqkv, A_wo, B_x, B_w_r, B_w_i):
    del B_x
    hbm = pl.BlockSpec(memory_space=pltpu.HBM)
    vmem = pl.BlockSpec(memory_space=pltpu.VMEM)
    out = pl.pallas_call(
        _kernel,
        out_shape=jax.ShapeDtypeStruct((S, D), BF16),
        in_specs=[hbm] * 6 + [vmem] * 6,
        out_specs=hbm,
        scratch_shapes=[
            pltpu.VMEM((NS, D, L), F32),
            pltpu.VMEM((8, S, L), BF16),
            pltpu.VMEM((4, D, D), BF16),
            pltpu.VMEM((4 * D, D), BF16),
            pltpu.VMEM((2, D // 2 + 1, S), BF16),
            pltpu.VMEM((4, 512, L), F32),
            pltpu.VMEM((2 * NS, FR, L), F32),
            pltpu.VMEM((NS, 2 * L, 2 * L), BF16),
            pltpu.VMEM((NS, D, L), BF16),
            pltpu.VMEM((D, L), F32),
            pltpu.VMEM((2 * NS, 2 * D, L), F32),
            pltpu.VMEM((NS, D, L), BF16),
            pltpu.VMEM((NS, FR, 2 * L), F32),
            pltpu.VMEM((NS, FR, 2 * L), BF16),
            pltpu.SemaphoreType.DMA((16,)),
        ],
        compiler_params=pltpu.CompilerParams(vmem_limit_bytes=124 * 1024 * 1024),
    )(A_x.reshape(S, D), A_wqkv, A_wo, B_w_r.T, B_w_i.T, *_CONSTS)
    return out.reshape(1, S, D)
```

```python
import numpy as np
import jax
import jax.numpy as jnp
from jax import lax
import jax.experimental.pallas as pl
import jax.experimental.pallas.tpu as pltpu

S, D, H, DH, WIN = 2048, 1024, 32, 32, 8
NS, L = 16, 128
FR = 528
F32, BF16 = jnp.float32, jnp.bfloat16
NT = (((1,), (1,)), ((), ()))


def _consts():
    i = np.arange(L)
    hs = []
    for n1 in range(NS):
        h = np.exp(-2j * np.pi * np.outer(n1 + NS * i, i) / S)
        hs.append(np.stack([h.real, h.imag - h.real, h.real + h.imag]))

    def e(r):
        return np.exp(-2j * np.pi * np.outer(r + 8 * np.arange(64), i) / D)

    ny = np.zeros((16, L))
    ny[0] = np.cos(np.pi * i)
    g0 = np.concatenate([e(0).real, e(0).imag, ny])
    g4 = np.concatenate([e(4).real, e(4).imag])
    gc = []
    for r, sg in ((1, -1.0), (2, -1.0), (3, 1.0)):
        a, b = e(r), e(8 - r)
        gc.append(np.block([[a.real, -sg * a.imag], [b.real, sg * b.imag],
                            [a.imag, sg * a.real], [b.imag, -sg * b.real]]))
    gc = np.stack(gc)
    out = (np.stack(hs), g0, g4, gc, g0.T, g4.T, gc.transpose(0, 2, 1))
    return tuple(np.ascontiguousarray(o).astype(BF16) for o in out)


_CONSTS = _consts()


def _cmul(xr, xi, k, n):
    c, s = np.cos(2 * np.pi * k / n), np.sin(2 * np.pi * k / n)
    if abs(abs(c) - abs(s)) < 1e-12:
        c = np.float32(c)
        if c * s > 0:
            return (xr - xi) * c, (xr + xi) * c
        return (xr + xi) * c, (xi - xr) * c
    c, s = np.float32(c), np.float32(s)
    return xr * c - xi * s, xr * s + xi * c


def _fft(x, sg):
    n = len(x)
    if n == 1:
        return x
    ev, od = _fft(x[0::2], sg), _fft(x[1::2], sg)
    lo, hi = [], []
    for k in range(n // 2):
        (er, ei), (tr, ti) = ev[k], od[k]
        if 4 * k == n:
            p, m = (er - ti, ei + tr), (er + ti, ei - tr)
            p, m = (p, m) if sg > 0 else (m, p)
        else:
            if k:
                tr, ti = _cmul(tr, ti, sg * k, n)
            p, m = (er + tr, ei + ti), (er - tr, ei - ti)
        lo.append(p)
        hi.append(m)
    return lo + hi


def _dot(a, b):
    return jnp.dot(a, b, preferred_element_type=F32)


def _layernorm(x):
    m = jnp.sum(x, axis=0, keepdims=True) * (1.0 / D)
    c = x - m
    v = jnp.sum(c * c, axis=0, keepdims=True) * (1.0 / D)
    return c * lax.rsqrt(v + 1e-5)


def _interleave(*gens):
    gens = list(gens)
    while gens:
        gens = [g for g in gens if next(g, 0) is None]


def _kernel(x_hbm, wqkv_hbm, wo_hbm, wr_hbm, wi_hbm, hs_hbm, g0, g4, gc, a0, a4, ac,
            out_hbm, xt, xb, wraw, wt, fraw, fst, filt, hs, xn, q, kv, ot, yf, yb, sems):
    col = lambda c, n=L: pl.ds(c * n, n)
    cp_w = [pltpu.make_async_copy(wqkv_hbm.at[:, col(c, D)], wraw.at[c], sems.at[c])
            for c in range(3)]
    cp_w.append(pltpu.make_async_copy(wo_hbm, wraw.at[3], sems.at[3]))
    cp_r = [pltpu.make_async_copy(wr_hbm, fraw.at[0], sems.at[4]),
            pltpu.make_async_copy(wi_hbm, fraw.at[1], sems.at[5]),
            pltpu.make_async_copy(hs_hbm, hs, sems.at[6])]
    cp_x = [pltpu.make_async_copy(x_hbm.at[:, col(c)], xb.at[c], sems.at[8 + c])
            for c in range(8)]
    for c in cp_w[1:3] + cp_x:
        c.start()
    xw = xb.bitcast(jnp.int32)

    with jax.named_scope("prep"):
        for b in (1, 2):
            cp_w[b].wait()
            for c in range(8):
                wt[col(8 * b + c, 64), :] = pltpu.bitcast(wraw[b, :, col(c)].T, jnp.int32)
        for c in range(8):
            cp_x[c].wait()
            if c == 5:
                for d in [cp_w[0], cp_w[3]] + cp_r:
                    d.start()
            for j in range(NS // 2):
                w = xw[c, pl.ds(j, L, stride=NS // 2), :].T
                xt[2 * j, col(c), :] = lax.bitcast_convert_type(w << 16, F32)
                xt[2 * j + 1, col(c), :] = lax.bitcast_convert_type(w & -65536, F32)

    lane = lax.broadcasted_iota(jnp.int32, (8, L), 1)
    cc = np.float32(np.sqrt(0.5))
    CH = 4
    RC = D // CH
    wrows = lambda c: pltpu.bitcast(wt[col(c, RC // 2), :], BF16)

    def prep_rest(t):
        o = pl.ds(pl.multiple_of(t * L, L), L)
        for b in (0, 3):
            wt[pl.ds(pl.multiple_of(b * 512 + t * 64, 64), 64), :] = pltpu.bitcast(
                wraw[b, :, o].T, jnp.int32)
            yield
        sc = np.float32(2.0 / (S * D))
        sc0 = jnp.where(lax.broadcasted_iota(jnp.int32, (64, L), 0) == 0, sc * 0.5, sc)
        row16 = lax.broadcasted_iota(jnp.int32, (16, L), 0)
        for p in range(2):
            for e in range(2):
                k1 = 2 * t + e
                cs = pl.ds(pl.multiple_of(k1 * L, L), L)
                fst[2 * p + e] = fraw[p, 0:512, cs].astype(F32)
                for b in range(8):
                    filt[p * NS + k1, col(b, 64), :] = (
                        fst[2 * p + e, pl.ds(b, 64, stride=8), :] * (sc0 if b == 0 else sc))
                ny = jnp.broadcast_to(fraw[p, 512:513, cs].astype(F32), (16, L))
                filt[p * NS + k1, 512:FR, :] = jnp.where(row16 == 0, ny * (sc * 0.5), 0.0)
                yield

    def ln_in(n1):
        yield
        xn[n1] = _layernorm(xt[n1]).astype(BF16)

    def kv_proj(n1):
        xv = xn[n1]
        for c in range(2 * CH):
            t = _dot(wrows(CH + c), xv)
            kv[NS + n1, col(c, RC), :] = t
            kv[n1, col(c, RC), :] = pltpu.roll(t, 1, 1)
            yield

    def q_proj(n1):
        xv = xn[n1]
        for c in range(CH):
            yield
            q[col(c, RC), :] = _dot(wrows(c), xv) * np.float32(DH ** -0.5)
            yield

    def attn(n1):
        for h in range(H):
            r = col(h, DH)
            qh = q[r, :]
            lg = []
            for w in range(WIN):
                p = qh * kv[NS + n1 - 2 * w, r, :]
                p = (p[0:8] + p[8:16]) + (p[16:24] + p[24:32])
                for sh in (4, 2, 1):
                    p = p + pltpu.roll(p, sh, 0)
                if w:
                    p = jnp.where((lane > 0) | (n1 >= 2 * w), p, -1e9)
                lg.append(p)
            mx = lg[0]
            for p in lg[1:]:
                mx = jnp.maximum(mx, p)
            ex = [jnp.exp(p - mx) for p in lg]
            sm = ex[0]
            for p in ex[1:]:
                sm = sm + p
            inv = 1.0 / sm
            o = None
            for w in range(WIN):
                t = kv[NS + n1 - 2 * w, col(H + h, DH), :].reshape(4, 8, L) * ex[w][None]
                o = t if o is None else o + t
            ot[n1, r, :] = (o * inv[None]).reshape(DH, L).astype(BF16)
            if h % 4 == 3:
                yield

    def out_proj(n1):
        ov = ot[n1]
        for c in range(CH):
            xt[n1, col(c, RC), :] += _dot(wrows(3 * CH + c), ov)
            yield
            yield

    def fwd(n1):
        x = _layernorm(xt[n1])
        yield
        xs = [x[j * L:(j + 1) * L] for j in range(8)]
        a = [xs[j] + xs[j + 4] for j in range(4)]
        b = [xs[j] - xs[j + 4] for j in range(4)]
        ev, od = a[0] + a[2], a[1] + a[3]
        t1, t2 = (b[1] - b[3]) * cc, (b[1] + b[3]) * cc
        yield
        z0 = _dot(g0[...], (ev + od).astype(BF16))
        z4 = _dot(g4[...], (ev - od).astype(BF16))
        zc = []
        for k, (ur, ui) in enumerate(((b[0] + t1, b[2] + t2), (a[0] - a[2], a[1] - a[3]),
                                      (b[0] - t1, b[2] - t2))):
            yield
            u = jnp.concatenate([ur.astype(BF16), ui.astype(BF16)], axis=0)
            zc.append(_dot(gc[k], u))
        parts = []
        for o in (0, 1):
            parts.append(jnp.concatenate(
                [z0[o * 64:o * 64 + 64]] + [zc[k][o * L:o * L + 64] for k in range(3)]
                + [z4[o * 64:o * 64 + 64]] + [zc[k][o * L + 64:o * L + L] for k in (2, 1, 0)]
                + [z0[L:L + 16] if o == 0 else jnp.zeros((16, L), F32)], axis=0))
        yield
        k1 = _dot((parts[0] + parts[1]).astype(BF16), hs[n1, 0])
        yf[n1, 0] = k1 - _dot(parts[1].astype(BF16), hs[n1, 2])
        yf[n1, 1] = k1 + _dot(parts[0].astype(BF16), hs[n1, 1])

    def mid(i):
        res = []
        for hf in range(2):
            r = pl.ds(pl.multiple_of(i * 16 + hf * 8, 8), 8)
            z = _fft([(yf[j, 0, r, :], yf[j, 1, r, :]) for j in range(NS)], -1)
            u = []
            for j, (zr, zi) in enumerate(z):
                fr, fi = filt[j, r, :], filt[NS + j, r, :]
                u.append((zr * fr - zi * fi, zr * fi + zi * fr))
            res.append([(a, b, a + b) for a, b in _fft(u, 1)])
        r = pl.ds(pl.multiple_of(i * 16, 16), 16)
        for j in range(NS):
            for o in range(3):
                yb[j, o, r, :] = jnp.concatenate(
                    [res[0][j][o], res[1][j][o]], axis=0).astype(BF16)

    def inv(n1):
        k1, k2, k3 = [lax.dot_general(yb[n1, i], hs[n1, j], NT, preferred_element_type=F32)
                      for i, j in ((2, 0), (0, 2), (1, 1))]
        z = ((k1 + k3).astype(BF16), (k1 - k2).astype(BF16))
        blk = lambda r, o: z[o][r * 64:r * 64 + 64]
        yield
        v0 = _dot(a0[...], jnp.concatenate([blk(0, 0), blk(0, 1), z[0][512:FR]], axis=0))
        v4 = _dot(a4[...], jnp.concatenate([blk(4, 0), blk(4, 1)], axis=0))
        vc = []
        for k in range(3):
            yield
            vc.append(_dot(ac[k], jnp.concatenate(
                [blk(k + 1, 0), blk(7 - k, 0), blk(k + 1, 1), blk(7 - k, 1)], axis=0)))
        yield
        (v1r, v1i), (v2r, v2i), (v3r, v3i) = [(v[0:L], v[L:2 * L]) for v in vc]
        ev, od = v0 + v4, v0 - v4
        a = [ev + v2r, od + v2i, ev - v2r, od - v2i]
        t1, t2 = v1r - v3r, v1i - v3i
        b = [v1r + v3r, (t1 + t2) * cc, v1i + v3i, (t2 - t1) * cc]
        for j in range(4):
            xt[n1, col(j), :] += a[j] + b[j]
            xt[n1, col(j + 4), :] += a[j] - b[j]

    def pipeline(name, stages, cuts=()):
        end = max(g + n for _, g, n in stages)
        pts = sorted({0, end, *cuts, *[g for _, g, _ in stages], *[g + n for _, g, n in stages]})
        with jax.named_scope(name):
            for lo, hi in zip(pts, pts[1:]):
                if lo in cuts:
                    for d in [cp_w[0], cp_w[3]] + cp_r:
                        d.wait()

                def body(t, lo=lo):
                    _interleave(*[fn(t - g) for fn, g, n in stages if g <= lo < g + n])
                if hi - lo == 1:
                    body(lo)
                else:
                    pl.loop(lo, hi)(body)

    for layer in range(2):
        if layer == 0:
            pipeline("kv0", [(kv_proj, 1, NS), (ln_in, 0, NS), (prep_rest, 7, 8),
                             (q_proj, NS, 1)], cuts=(7,))
        else:
            pipeline("kv1", [(kv_proj, 2, NS), (ln_in, 1, NS), (inv, 0, NS), (q_proj, NS + 1, 1)])
        pipeline("att", [(fwd, 2, NS), (out_proj, 1, NS), (attn, 0, NS),
                         (lambda t: q_proj(t + 1), 0, NS - 1)])
        with jax.named_scope("mid"):
            pl.loop(0, FR // 16)(mid)
    with jax.named_scope("inv"):
        pl.loop(0, NS // 2)(lambda t: _interleave(inv(2 * t), inv(2 * t + 1)))

    with jax.named_scope("out"):
        cp_o = [pltpu.make_async_copy(xb.at[c], out_hbm.at[:, col(c)], sems.at[8 + c])
                for c in range(8)]
        bits = lambda v: lax.bitcast_convert_type(v.astype(BF16).astype(F32), jnp.int32)
        for c in range(8):
            for j in range(NS // 2):
                w = (lax.shift_right_logical(bits(xt[2 * j, col(c), :]), 16)
                     | bits(xt[2 * j + 1, col(c), :]))
                xw[c, pl.ds(j, L, stride=NS // 2), :] = w.T
            cp_o[c].start()
        for d in cp_o:
            d.wait()


@jax.jit
def pallas_interleave_layers__sliding_local_dilated__spectral_gfnet__prompt_kernel(
        A_x, A_wqkv, A_wo, B_x, B_w_r, B_w_i):
    del B_x
    hbm = pl.BlockSpec(memory_space=pltpu.HBM)
    vmem = pl.BlockSpec(memory_space=pltpu.VMEM)
    out = pl.pallas_call(
        _kernel,
        out_shape=jax.ShapeDtypeStruct((S, D), BF16),
        in_specs=[hbm] * 6 + [vmem] * 6,
        out_specs=hbm,
        scratch_shapes=[
            pltpu.VMEM((NS, D, L), F32),
            pltpu.VMEM((8, S, L), BF16),
            pltpu.VMEM((4, D, D), BF16),
            pltpu.VMEM((2 * D, D), jnp.int32),
            pltpu.VMEM((2, D // 2 + 1, S), BF16),
            pltpu.VMEM((4, 512, L), F32),
            pltpu.VMEM((2 * NS, FR, L), F32),
            pltpu.VMEM((NS, 3, L, L), BF16),
            pltpu.VMEM((NS, D, L), BF16),
            pltpu.VMEM((D, L), F32),
            pltpu.VMEM((2 * NS, 2 * D, L), F32),
            pltpu.VMEM((NS, D, L), BF16),
            pltpu.VMEM((NS, 2, FR, L), F32),
            pltpu.VMEM((NS, 3, FR, L), BF16),
            pltpu.SemaphoreType.DMA((16,)),
        ],
        compiler_params=pltpu.CompilerParams(vmem_limit_bytes=124 * 1024 * 1024),
    )(A_x.reshape(S, D), A_wqkv, A_wo, B_w_r.T, B_w_i.T, *_CONSTS)
    return out.reshape(1, S, D)
```

```python
import numpy as np
import jax
import jax.numpy as jnp
from jax import lax
import jax.experimental.pallas as pl
import jax.experimental.pallas.tpu as pltpu

S, D, H, DH, WIN = 2048, 1024, 32, 32, 8
NS, L = 16, 128
FR = 528
F32, BF16 = jnp.float32, jnp.bfloat16
NT = (((1,), (1,)), ((), ()))


def _consts():
    i = np.arange(L)
    hs = []
    for n1 in range(NS):
        h = np.exp(-2j * np.pi * np.outer(n1 + NS * i, i) / S)
        hs.append(np.stack([h.real, h.imag - h.real, h.real + h.imag]))

    def e(r):
        return np.exp(-2j * np.pi * np.outer(r + 8 * np.arange(64), i) / D)

    ny = np.zeros((16, L))
    ny[0] = np.cos(np.pi * i)
    g0 = np.concatenate([e(0).real, e(0).imag, ny])
    g4 = np.concatenate([e(4).real, e(4).imag])
    gc = []
    for r, sg in ((1, -1.0), (2, -1.0), (3, 1.0)):
        a, b = e(r), e(8 - r)
        gc.append(np.block([[a.real, -sg * a.imag], [b.real, sg * b.imag],
                            [a.imag, sg * a.real], [b.imag, -sg * b.real]]))
    gc = np.stack(gc)
    out = (np.stack(hs), g0, g4, gc, g0.T, g4.T, gc.transpose(0, 2, 1))
    return tuple(np.ascontiguousarray(o).astype(BF16) for o in out)


_CONSTS = _consts()


def _cmul(xr, xi, k, n):
    c, s = np.cos(2 * np.pi * k / n), np.sin(2 * np.pi * k / n)
    if abs(abs(c) - abs(s)) < 1e-12:
        c = np.float32(c)
        if c * s > 0:
            return (xr - xi) * c, (xr + xi) * c
        return (xr + xi) * c, (xi - xr) * c
    c, s = np.float32(c), np.float32(s)
    return xr * c - xi * s, xr * s + xi * c


def _fft(x, sg):
    n = len(x)
    if n == 1:
        return x
    ev, od = _fft(x[0::2], sg), _fft(x[1::2], sg)
    lo, hi = [], []
    for k in range(n // 2):
        (er, ei), (tr, ti) = ev[k], od[k]
        if 4 * k == n:
            p, m = (er - ti, ei + tr), (er + ti, ei - tr)
            p, m = (p, m) if sg > 0 else (m, p)
        else:
            if k:
                tr, ti = _cmul(tr, ti, sg * k, n)
            p, m = (er + tr, ei + ti), (er - tr, ei - ti)
        lo.append(p)
        hi.append(m)
    return lo + hi


def _dot(a, b):
    return jnp.dot(a, b, preferred_element_type=F32)


def _interleave(*gens):
    gens = [[0.0, g] for g in gens]
    while gens:
        e = min(gens, key=lambda v: v[0])
        e[0] = next(e[1], None)
        gens = [v for v in gens if v[0] is not None]


def _kernel(x_hbm, wqkv_hbm, wo_hbm, wr_hbm, wi_hbm, hs_hbm, g0, g4, gc, a0, a4, ac,
            out_hbm, xt, xb, wraw, wt, fraw, fst, filt, hs, xn, q, ub, kv, ot, yf, yb, sems):
    col = lambda c, n=L: pl.ds(c * n, n)
    cp_w = [pltpu.make_async_copy(wqkv_hbm.at[:, col(c, D)], wraw.at[c], sems.at[c])
            for c in range(3)]
    cp_w.append(pltpu.make_async_copy(wo_hbm, wraw.at[3], sems.at[3]))
    cp_r = [pltpu.make_async_copy(wr_hbm, fraw.at[0], sems.at[4]),
            pltpu.make_async_copy(wi_hbm, fraw.at[1], sems.at[5]),
            pltpu.make_async_copy(hs_hbm, hs, sems.at[6])]
    cp_x = [pltpu.make_async_copy(x_hbm.at[:, col(c)], xb.at[c], sems.at[8 + c])
            for c in range(8)]
    for c in cp_w[1:3] + cp_x:
        c.start()
    xw = xb.bitcast(jnp.int32)

    with jax.named_scope("prep"):
        for b in (1, 2):
            cp_w[b].wait()
            for c in range(8):
                wt[col(8 * b + c, 64), :] = pltpu.bitcast(wraw[b, :, col(c)].T, jnp.int32)
        for c in range(8):
            cp_x[c].wait()
            if c == 5:
                for d in [cp_w[0], cp_w[3]] + cp_r:
                    d.start()
            for j in range(NS // 2):
                w = xw[c, pl.ds(j, L, stride=NS // 2), :].T
                xt[2 * j, col(c), :] = lax.bitcast_convert_type(w << 16, F32)
                xt[2 * j + 1, col(c), :] = lax.bitcast_convert_type(w & -65536, F32)

    lane = lax.broadcasted_iota(jnp.int32, (8, L), 1)
    sub = lax.broadcasted_iota(jnp.int32, (8, L), 0)
    cc = np.float32(np.sqrt(0.5))
    CH = 8
    RC = D // CH
    wrows = lambda c, n: pltpu.bitcast(wt[col(c, n // 2), :], BF16)

    def prep_rest(t):
        o = pl.ds(pl.multiple_of(t * L, L), L)
        for b in (0, 3):
            wt[pl.ds(pl.multiple_of(b * 512 + t * 64, 64), 64), :] = pltpu.bitcast(
                wraw[b, :, o].T, jnp.int32)
            yield 0.1 + 0.05 * b
        sc = np.float32(2.0 / (S * D))
        sc0 = jnp.where(lax.broadcasted_iota(jnp.int32, (64, L), 0) == 0, sc * 0.5, sc)
        row16 = lax.broadcasted_iota(jnp.int32, (16, L), 0)
        for p in range(2):
            for e in range(2):
                k1 = 2 * t + e
                cs = pl.ds(pl.multiple_of(k1 * L, L), L)
                fst[2 * p + e] = fraw[p, 0:512, cs].astype(F32)
                for b in range(8):
                    filt[p * NS + k1, col(b, 64), :] = (
                        fst[2 * p + e, pl.ds(b, 64, stride=8), :] * (sc0 if b == 0 else sc))
                ny = jnp.broadcast_to(fraw[p, 512:513, cs].astype(F32), (16, L))
                filt[p * NS + k1, 512:FR, :] = jnp.where(row16 == 0, ny * (sc * 0.5), 0.0)
                yield 0.4 + 0.3 * p + 0.15 * e

    def stats(n1, p0, dp):
        acc = 0.0
        for j in range(8):
            yield p0 + j * dp
            acc = acc + xt[n1, col(j), :].reshape(L // 16, 16, L).sum(axis=0)
        m = jnp.sum(acc, axis=0, keepdims=True) * (1.0 / D)
        acc = 0.0
        for j in range(8):
            yield p0 + (8 + j) * dp
            c = xt[n1, col(j), :] - m
            acc = acc + (c * c).reshape(L // 16, 16, L).sum(axis=0)
        return m, lax.rsqrt(jnp.sum(acc, axis=0, keepdims=True) * (1.0 / D) + 1e-5)

    def ln_in(n1):
        m, r = yield from stats(n1, 0.02, 0.03)
        for j in range(8):
            yield 0.55 + 0.04 * j
            xn[n1, col(j), :] = ((xt[n1, col(j), :] - m) * r).astype(BF16)

    def kv_proj(n1, n=256):
        xv = xn[n1]
        for c in range(2 * D // n):
            yield c * n / (2 * D)
            t = _dot(wrows(D // n + c, n), xv)
            kv[NS + n1, col(c, n), :] = t
            kv[n1, col(c, n), :] = pltpu.roll(t, 1, 1)

    def q_proj(n1):
        xv = xn[n1]
        for c in range(CH):
            yield (c + 1) / CH
            q[col(c, RC), :] = _dot(wrows(c, RC), xv) * np.float32(DH ** -0.5)

    def attn(n1):
        valid = (lane > 0) | (2 * sub <= n1)
        for h in range(H):
            yield (h + 0.5) / H
            r = col(h, DH)
            qh = q[r, :]
            lg = []
            for w in range(WIN):
                p = qh * kv[NS + n1 - 2 * w, r, :]
                lg.append((p[0:8] + p[8:16]) + (p[16:24] + p[24:32]))
            for sh in (1, 2, 4):
                m = (sub & sh) == 0
                lg = [jnp.where(m, a, b) + pltpu.roll(jnp.where(m, b, a), 8 - sh, 0)
                      for a, b in zip(lg[0::2], lg[1::2])]
            p = jnp.where(valid, lg[0], -1e9)
            mx = p
            for sh in (4, 2, 1):
                mx = jnp.maximum(mx, pltpu.roll(mx, sh, 0))
            e = jnp.exp(p - mx)
            sm = e
            for sh in (4, 2, 1):
                sm = sm + pltpu.roll(sm, sh, 0)
            e = e / sm
            o = None
            for w in range(WIN):
                t = kv[NS + n1 - 2 * w, col(H + h, DH), :] * e[w:w + 1]
                o = t if o is None else o + t
            ot[n1, r, :] = o.astype(BF16)

    def out_proj(n1):
        ov = ot[n1]
        for c in range(CH):
            yield (c + 0.4 * (c > 0)) / CH
            xt[n1, col(c, RC), :] += _dot(wrows(3 * CH + c, RC), ov)

    def fwd(n1):
        m, r = yield from stats(n1, 0.01, 0.02)
        for i in range(8):
            yield 0.4 + 0.07 * i
            xs = [(xt[n1, col(8 * j + i, 16), :] - m) * r for j in range(8)]
            a = [xs[j] + xs[j + 4] for j in range(4)]
            b = [xs[j] - xs[j + 4] for j in range(4)]
            ev, od = a[0] + a[2], a[1] + a[3]
            t1, t2 = (b[1] - b[3]) * cc, (b[1] + b[3]) * cc
            for j, u in enumerate((b[0] + t1, b[2] + t2, a[0] - a[2], a[1] - a[3],
                                   b[0] - t1, b[2] - t2, ev + od, ev - od)):
                ub[col(8 * j + i, 16), :] = u.astype(BF16)

    def fwd_d(n1):
        yield 0.1
        z0 = _dot(g0[...], ub[col(6), :])
        z4 = _dot(g4[...], ub[col(7), :])
        zc = [_dot(gc[k], ub[col(k, 256), :]) for k in range(3)]
        parts = []
        for o in (0, 1):
            parts.append(jnp.concatenate(
                [z0[o * 64:o * 64 + 64]] + [zc[k][o * L:o * L + 64] for k in range(3)]
                + [z4[o * 64:o * 64 + 64]] + [zc[k][o * L + 64:o * L + L] for k in (2, 1, 0)]
                + [z0[L:L + 16] if o == 0 else jnp.zeros((16, L), F32)], axis=0))
        for o, v in enumerate(parts + [parts[0] + parts[1]]):
            yb[n1, o] = v.astype(BF16)

    def fwd_s(n1):
        k1 = _dot(yb[n1, 2], hs[n1, 0])
        yf[n1, 0] = k1 - _dot(yb[n1, 1], hs[n1, 2])
        yf[n1, 1] = k1 + _dot(yb[n1, 0], hs[n1, 1])
        yield 1.0

    def mid(i):
        res = []
        for hf in range(2):
            r = pl.ds(pl.multiple_of(i * 16 + hf * 8, 8), 8)
            z = _fft([(yf[j, 0, r, :], yf[j, 1, r, :]) for j in range(NS)], -1)
            u = []
            for j, (zr, zi) in enumerate(z):
                fr, fi = filt[j, r, :], filt[NS + j, r, :]
                u.append((zr * fr - zi * fi, zr * fi + zi * fr))
            res.append([(a, b, a + b) for a, b in _fft(u, 1)])
        r = pl.ds(pl.multiple_of(i * 16, 16), 16)
        for j in range(NS):
            for o in range(3):
                yb[j, o, r, :] = jnp.concatenate(
                    [res[0][j][o], res[1][j][o]], axis=0).astype(BF16)

    def inv(n1):
        k1, k2, k3 = [lax.dot_general(yb[n1, i], hs[n1, j], NT, preferred_element_type=F32)
                      for i, j in ((2, 0), (0, 2), (1, 1))]
        z = ((k1 + k3).astype(BF16), (k1 - k2).astype(BF16))
        blk = lambda r, o: z[o][r * 64:r * 64 + 64]
        yield 0.2
        v0 = _dot(a0[...], jnp.concatenate([blk(0, 0), blk(0, 1), z[0][512:FR]], axis=0))
        v4 = _dot(a4[...], jnp.concatenate([blk(4, 0), blk(4, 1)], axis=0))
        vc = []
        for k in range(3):
            yield 0.3 + 0.12 * k
            vc.append(_dot(ac[k], jnp.concatenate(
                [blk(k + 1, 0), blk(7 - k, 0), blk(k + 1, 1), blk(7 - k, 1)], axis=0)))
        for i in range(8):
            yield 0.58 + 0.045 * i
            (v1r, v1i), (v2r, v2i), (v3r, v3i) = [
                (v[16 * i:16 * i + 16], v[L + 16 * i:L + 16 * i + 16]) for v in vc]
            u0, u4 = v0[16 * i:16 * i + 16], v4[16 * i:16 * i + 16]
            ev, od = u0 + u4, u0 - u4
            a = [ev + v2r, od + v2i, ev - v2r, od - v2i]
            t1, t2 = v1r - v3r, v1i - v3i
            b = [v1r + v3r, (t1 + t2) * cc, v1i + v3i, (t2 - t1) * cc]
            for j in range(4):
                xt[n1, col(8 * j + i, 16), :] += a[j] + b[j]
                xt[n1, col(8 * j + 32 + i, 16), :] += a[j] - b[j]

    def pipeline(name, stages, cuts=()):
        end = max(g + n for _, g, n in stages)
        pts = sorted({0, end, *cuts, *[g for _, g, _ in stages], *[g + n for _, g, n in stages]})
        with jax.named_scope(name):
            for lo, hi in zip(pts, pts[1:]):
                if lo in cuts:
                    for d in [cp_w[0], cp_w[3]] + cp_r:
                        d.wait()

                def body(t, lo=lo):
                    _interleave(*[fn(t - g) for fn, g, n in stages if g <= lo < g + n])
                if hi - lo == 1:
                    body(lo)
                else:
                    with jax.named_scope(f'{name}_{hi - lo}'):
                        pl.loop(lo, hi, unroll=1)(body)

    for layer in range(2):
        if layer == 0:
            pipeline("kv0", [(lambda t: kv_proj(t, D), 1, NS), (ln_in, 0, NS), (prep_rest, 7, 8),
                             (q_proj, NS, 1)], cuts=(7,))
        else:
            pipeline("kv1", [(kv_proj, 2, NS), (ln_in, 1, NS), (inv, 0, NS), (q_proj, NS + 1, 1)])
        pipeline("att", [(fwd_s, 4, NS), (fwd_d, 3, NS), (fwd, 2, NS), (out_proj, 1, NS), (attn, 0, NS),
                         (lambda t: q_proj(t + 1), 0, NS - 1)])
        with jax.named_scope("mid"):
            pl.loop(0, FR // 16)(mid)
    with jax.named_scope("inv"):
        pl.loop(0, NS // 2)(lambda t: _interleave(inv(2 * t), inv(2 * t + 1)))

    with jax.named_scope("out"):
        cp_o = [pltpu.make_async_copy(xb.at[c], out_hbm.at[:, col(c)], sems.at[8 + c])
                for c in range(8)]
        bits = lambda v: lax.bitcast_convert_type(v.astype(BF16).astype(F32), jnp.int32)
        for c in range(8):
            for j in range(NS // 2):
                w = (lax.shift_right_logical(bits(xt[2 * j, col(c), :]), 16)
                     | bits(xt[2 * j + 1, col(c), :]))
                xw[c, pl.ds(j, L, stride=NS // 2), :] = w.T
            cp_o[c].start()
        for d in cp_o:
            d.wait()


@jax.jit
def pallas_interleave_layers__sliding_local_dilated__spectral_gfnet__prompt_kernel(
        A_x, A_wqkv, A_wo, B_x, B_w_r, B_w_i):
    del B_x
    hbm = pl.BlockSpec(memory_space=pltpu.HBM)
    vmem = pl.BlockSpec(memory_space=pltpu.VMEM)
    out = pl.pallas_call(
        _kernel,
        out_shape=jax.ShapeDtypeStruct((S, D), BF16),
        in_specs=[hbm] * 6 + [vmem] * 6,
        out_specs=hbm,
        scratch_shapes=[
            pltpu.VMEM((NS, D, L), F32),
            pltpu.VMEM((8, S, L), BF16),
            pltpu.VMEM((4, D, D), BF16),
            pltpu.VMEM((2 * D, D), jnp.int32),
            pltpu.VMEM((2, D // 2 + 1, S), BF16),
            pltpu.VMEM((4, 512, L), F32),
            pltpu.VMEM((2 * NS, FR, L), F32),
            pltpu.VMEM((NS, 3, L, L), BF16),
            pltpu.VMEM((NS, D, L), BF16),
            pltpu.VMEM((D, L), F32),
            pltpu.VMEM((D, L), BF16),
            pltpu.VMEM((2 * NS, 2 * D, L), F32),
            pltpu.VMEM((NS, D, L), BF16),
            pltpu.VMEM((NS, 2, FR, L), F32),
            pltpu.VMEM((NS, 3, FR, L), BF16),
            pltpu.SemaphoreType.DMA((16,)),
        ],
        compiler_params=pltpu.CompilerParams(vmem_limit_bytes=124 * 1024 * 1024),
    )(A_x.reshape(S, D), A_wqkv, A_wo, B_w_r.T, B_w_i.T, *_CONSTS)
    return out.reshape(1, S, D)
```

```python
import numpy as np
import jax
import jax.numpy as jnp
from jax import lax
import jax.experimental.pallas as pl
import jax.experimental.pallas.tpu as pltpu

S, D, H, DH, WIN = 2048, 1024, 32, 32, 8
NS, L = 16, 128
FR = 528
F32, BF16 = jnp.float32, jnp.bfloat16
NT = (((1,), (1,)), ((), ()))


def _consts():
    i = np.arange(L)
    hs = []
    for n1 in range(NS):
        h = np.exp(-2j * np.pi * np.outer(n1 + NS * i, i) / S)
        hs.append(np.stack([h.real, h.imag - h.real, h.real + h.imag]))

    def e(r):
        return np.exp(-2j * np.pi * np.outer(r + 8 * np.arange(64), i) / D)

    ny = np.zeros((16, L))
    ny[0] = np.cos(np.pi * i)
    g0 = np.concatenate([e(0).real, e(0).imag, ny])
    g4 = np.concatenate([e(4).real, e(4).imag])
    gc = []
    for r, sg in ((1, -1.0), (2, -1.0), (3, 1.0)):
        a, b = e(r), e(8 - r)
        gc.append(np.block([[a.real, -sg * a.imag], [b.real, sg * b.imag],
                            [a.imag, sg * a.real], [b.imag, -sg * b.real]]))
    gc = np.stack(gc)
    out = (np.stack(hs), g0, g4, gc, g0.T, g4.T, gc.transpose(0, 2, 1))
    return tuple(np.ascontiguousarray(o).astype(BF16) for o in out)


_CONSTS = _consts()


def _cmul(xr, xi, k, n):
    c, s = np.cos(2 * np.pi * k / n), np.sin(2 * np.pi * k / n)
    if abs(abs(c) - abs(s)) < 1e-12:
        c = np.float32(c)
        if c * s > 0:
            return (xr - xi) * c, (xr + xi) * c
        return (xr + xi) * c, (xi - xr) * c
    c, s = np.float32(c), np.float32(s)
    return xr * c - xi * s, xr * s + xi * c


def _fft(x, sg):
    n = len(x)
    if n == 1:
        return x
    ev, od = _fft(x[0::2], sg), _fft(x[1::2], sg)
    lo, hi = [], []
    for k in range(n // 2):
        (er, ei), (tr, ti) = ev[k], od[k]
        if 4 * k == n:
            p, m = (er - ti, ei + tr), (er + ti, ei - tr)
            p, m = (p, m) if sg > 0 else (m, p)
        else:
            if k:
                tr, ti = _cmul(tr, ti, sg * k, n)
            p, m = (er + tr, ei + ti), (er - tr, ei - ti)
        lo.append(p)
        hi.append(m)
    return lo + hi


def _dot(a, b):
    return jnp.dot(a, b, preferred_element_type=F32)


def _interleave(*gens):
    gens = [[0.0, g] for g in gens]
    while gens:
        e = min(gens, key=lambda v: v[0])
        e[0] = next(e[1], None)
        gens = [v for v in gens if v[0] is not None]


def _kernel(x_hbm, wqkv_hbm, wo_hbm, wr_hbm, wi_hbm, hs_hbm, g0, g4, gc, a0, a4, ac,
            out_hbm, xt, xb, wraw, wt, fraw, fst, filt, hs, xn, q, ub, kv, ot, yf, yb, sems):
    col = lambda c, n=L: pl.ds(c * n, n)
    cp_w = [pltpu.make_async_copy(wqkv_hbm.at[:, col(c, D)], wraw.at[c], sems.at[c])
            for c in range(3)]
    cp_w.append(pltpu.make_async_copy(wo_hbm, wraw.at[3], sems.at[3]))
    cp_r = [pltpu.make_async_copy(wr_hbm, fraw.at[0], sems.at[4]),
            pltpu.make_async_copy(wi_hbm, fraw.at[1], sems.at[5]),
            pltpu.make_async_copy(hs_hbm, hs, sems.at[6])]
    cp_x = [pltpu.make_async_copy(x_hbm.at[:, col(c)], xb.at[c], sems.at[8 + c])
            for c in range(8)]
    for c in cp_w[1:3] + cp_x:
        c.start()
    xw = xb.bitcast(jnp.int32)

    with jax.named_scope("prep"):
        for b in (1, 2):
            cp_w[b].wait()
            for c in range(8):
                wt[col(8 * b + c, 64), :] = pltpu.bitcast(wraw[b, :, col(c)].T, jnp.int32)
        for c in range(8):
            cp_x[c].wait()
            if c == 5:
                for d in [cp_w[0], cp_w[3]] + cp_r:
                    d.start()
            for j in range(NS // 2):
                w = xw[c, pl.ds(j, L, stride=NS // 2), :].T
                xt[2 * j, col(c), :] = lax.bitcast_convert_type(w << 16, F32)
                xt[2 * j + 1, col(c), :] = lax.bitcast_convert_type(w & -65536, F32)

    lane = lax.broadcasted_iota(jnp.int32, (8, L), 1)
    sub = lax.broadcasted_iota(jnp.int32, (8, L), 0)
    cc = np.float32(np.sqrt(0.5))
    CH = 8
    RC = D // CH
    wrows = lambda c, n: pltpu.bitcast(wt[col(c, n // 2), :], BF16)

    def prep_rest(t):
        o = pl.ds(pl.multiple_of(t * L, L), L)
        for b in (0, 3):
            wt[pl.ds(pl.multiple_of(b * 512 + t * 64, 64), 64), :] = pltpu.bitcast(
                wraw[b, :, o].T, jnp.int32)
            yield 0.1 + 0.05 * b
        sc = np.float32(2.0 / (S * D))
        sc0 = jnp.where(lax.broadcasted_iota(jnp.int32, (64, L), 0) == 0, sc * 0.5, sc)
        row16 = lax.broadcasted_iota(jnp.int32, (16, L), 0)
        for p in range(2):
            for e in range(2):
                k1 = 2 * t + e
                cs = pl.ds(pl.multiple_of(k1 * L, L), L)
                fst[2 * p + e] = fraw[p, 0:512, cs].astype(F32)
                for b in range(8):
                    filt[p * NS + k1, col(b, 64), :] = (
                        fst[2 * p + e, pl.ds(b, 64, stride=8), :] * (sc0 if b == 0 else sc))
                ny = jnp.broadcast_to(fraw[p, 512:513, cs].astype(F32), (16, L))
                filt[p * NS + k1, 512:FR, :] = jnp.where(row16 == 0, ny * (sc * 0.5), 0.0)
                yield 0.4 + 0.3 * p + 0.15 * e

    def stats(n1, p0, dp):
        acc = 0.0
        for j in range(8):
            yield p0 + j * dp
            acc = acc + xt[n1, col(j), :].reshape(L // 16, 16, L).sum(axis=0)
        m = jnp.sum(acc, axis=0, keepdims=True) * (1.0 / D)
        acc = 0.0
        for j in range(8):
            yield p0 + (8 + j) * dp
            c = xt[n1, col(j), :] - m
            acc = acc + (c * c).reshape(L // 16, 16, L).sum(axis=0)
        return m, lax.rsqrt(jnp.sum(acc, axis=0, keepdims=True) * (1.0 / D) + 1e-5)

    def ln_in(n1):
        m, r = yield from stats(n1, 0.02, 0.03)
        for j in range(8):
            yield 0.55 + 0.04 * j
            xn[n1, col(j), :] = ((xt[n1, col(j), :] - m) * r).astype(BF16)

    def kv_proj(n1, n=256):
        xv = xn[n1]
        for c in range(2 * D // n):
            yield c * n / (2 * D)
            t = _dot(wrows(D // n + c, n), xv)
            kv[NS + n1, col(c, n), :] = t
            kv[n1, col(c, n), :] = pltpu.roll(t, 1, 1)

    def q_proj(n1):
        xv = xn[n1]
        for c in range(CH):
            yield (c + 1) / CH
            q[col(c, RC), :] = _dot(wrows(c, RC), xv) * np.float32(DH ** -0.5)

    def attn(n1):
        valid = (lane > 0) | (2 * sub <= n1)
        for h in range(H):
            yield (h + 0.5) / H
            r = col(h, DH)
            qh = q[r, :]
            lg = []
            for w in range(WIN):
                p = qh * kv[NS + n1 - 2 * w, r, :]
                lg.append((p[0:8] + p[8:16]) + (p[16:24] + p[24:32]))
            for sh in (1, 2, 4):
                m = (sub & sh) == 0
                lg = [jnp.where(m, a, b) + pltpu.roll(jnp.where(m, b, a), 8 - sh, 0)
                      for a, b in zip(lg[0::2], lg[1::2])]
            p = jnp.where(valid, lg[0], -1e9)
            mx = p
            for sh in (4, 2, 1):
                mx = jnp.maximum(mx, pltpu.roll(mx, sh, 0))
            e = jnp.exp(p - mx)
            sm = e
            for sh in (4, 2, 1):
                sm = sm + pltpu.roll(sm, sh, 0)
            e = e / sm
            o = None
            for w in range(WIN):
                t = kv[NS + n1 - 2 * w, col(H + h, DH), :] * e[w:w + 1]
                o = t if o is None else o + t
            ot[n1, r, :] = o.astype(BF16)

    def out_proj(n1):
        ov = ot[n1]
        for c in range(CH):
            yield (c + 0.4 * (c > 0)) / CH
            xt[n1, col(c, RC), :] += _dot(wrows(3 * CH + c, RC), ov)

    def fwd(n1):
        m, r = yield from stats(n1, 0.01, 0.02)
        for i in range(8):
            yield 0.4 + 0.07 * i
            xs = [(xt[n1, col(8 * j + i, 16), :] - m) * r for j in range(8)]
            a = [xs[j] + xs[j + 4] for j in range(4)]
            b = [xs[j] - xs[j + 4] for j in range(4)]
            ev, od = a[0] + a[2], a[1] + a[3]
            t1, t2 = (b[1] - b[3]) * cc, (b[1] + b[3]) * cc
            for j, u in enumerate((b[0] + t1, b[2] + t2, a[0] - a[2], a[1] - a[3],
                                   b[0] - t1, b[2] - t2, ev + od, ev - od)):
                ub[col(8 * j + i, 16), :] = u.astype(BF16)

    def fwd_d(n1):
        yield 0.1
        z0 = _dot(g0[...], ub[col(6), :])
        z4 = _dot(g4[...], ub[col(7), :])
        zc = [_dot(gc[k], ub[col(k, 256), :]) for k in range(3)]
        parts = []
        for o in (0, 1):
            parts.append(jnp.concatenate(
                [z0[o * 64:o * 64 + 64]] + [zc[k][o * L:o * L + 64] for k in range(3)]
                + [z4[o * 64:o * 64 + 64]] + [zc[k][o * L + 64:o * L + L] for k in (2, 1, 0)]
                + [z0[L:L + 16] if o == 0 else jnp.zeros((16, L), F32)], axis=0))
        for o, v in enumerate(parts + [parts[0] + parts[1]]):
            yb[n1, o] = v.astype(BF16)

    def fwd_s(n1):
        yield 0.6
        k1 = _dot(yb[n1, 2], hs[n1, 0])
        yf[n1, 0] = k1 - _dot(yb[n1, 1], hs[n1, 2])
        yf[n1, 1] = k1 + _dot(yb[n1, 0], hs[n1, 1])
        yield 1.0

    def mid(i):
        res = []
        for hf in range(2):
            r = pl.ds(pl.multiple_of(i * 16 + hf * 8, 8), 8)
            z = _fft([(yf[j, 0, r, :], yf[j, 1, r, :]) for j in range(NS)], -1)
            u = []
            for j, (zr, zi) in enumerate(z):
                fr, fi = filt[j, r, :], filt[NS + j, r, :]
                u.append((zr * fr - zi * fi, zr * fi + zi * fr))
            res.append([(a, b, a + b) for a, b in _fft(u, 1)])
        r = pl.ds(pl.multiple_of(i * 16, 16), 16)
        for j in range(NS):
            for o in range(3):
                yb[j, o, r, :] = jnp.concatenate(
                    [res[0][j][o], res[1][j][o]], axis=0).astype(BF16)

    def inv(n1):
        k1, k2, k3 = [lax.dot_general(yb[n1, i], hs[n1, j], NT, preferred_element_type=F32)
                      for i, j in ((2, 0), (0, 2), (1, 1))]
        z = ((k1 + k3).astype(BF16), (k1 - k2).astype(BF16))
        blk = lambda r, o: z[o][r * 64:r * 64 + 64]
        yield 0.2
        v0 = _dot(a0[...], jnp.concatenate([blk(0, 0), blk(0, 1), z[0][512:FR]], axis=0))
        v4 = _dot(a4[...], jnp.concatenate([blk(4, 0), blk(4, 1)], axis=0))
        vc = []
        for k in range(3):
            yield 0.3 + 0.12 * k
            vc.append(_dot(ac[k], jnp.concatenate(
                [blk(k + 1, 0), blk(7 - k, 0), blk(k + 1, 1), blk(7 - k, 1)], axis=0)))
        for i in range(8):
            yield 0.58 + 0.045 * i
            (v1r, v1i), (v2r, v2i), (v3r, v3i) = [
                (v[16 * i:16 * i + 16], v[L + 16 * i:L + 16 * i + 16]) for v in vc]
            u0, u4 = v0[16 * i:16 * i + 16], v4[16 * i:16 * i + 16]
            ev, od = u0 + u4, u0 - u4
            a = [ev + v2r, od + v2i, ev - v2r, od - v2i]
            t1, t2 = v1r - v3r, v1i - v3i
            b = [v1r + v3r, (t1 + t2) * cc, v1i + v3i, (t2 - t1) * cc]
            for j in range(4):
                xt[n1, col(8 * j + i, 16), :] += a[j] + b[j]
                xt[n1, col(8 * j + 32 + i, 16), :] += a[j] - b[j]

    def pipeline(name, stages, cuts=()):
        end = max(g + n for _, g, n in stages)
        pts = sorted({0, end, *cuts, *[g for _, g, _ in stages], *[g + n for _, g, n in stages]})
        with jax.named_scope(name):
            for lo, hi in zip(pts, pts[1:]):
                if lo in cuts:
                    for d in [cp_w[0], cp_w[3]] + cp_r:
                        d.wait()

                def body(t, lo=lo):
                    _interleave(*[fn(t - g) for fn, g, n in stages if g <= lo < g + n])
                if hi - lo == 1:
                    body(lo)
                else:
                    with jax.named_scope(f'{name}_{hi - lo}'):
                        pl.loop(lo, hi)(body)

    for layer in range(2):
        if layer == 0:
            pipeline("kv0", [(lambda t: kv_proj(t, D), 1, NS), (ln_in, 0, NS), (prep_rest, 7, 8),
                             (q_proj, NS, 1)], cuts=(7,))
        else:
            pipeline("kv1", [(kv_proj, 2, NS), (ln_in, 1, NS), (inv, 0, NS), (q_proj, NS + 1, 1)])
        pipeline("att", [(fwd_s, 3, NS), (fwd_d, 3, NS), (fwd, 2, NS), (out_proj, 1, NS), (attn, 0, NS),
                         (lambda t: q_proj(t + 1), 0, NS - 1)])
        with jax.named_scope("mid"):
            pl.loop(0, FR // 16)(mid)
    with jax.named_scope("inv"):
        pl.loop(0, NS // 4)(lambda t: _interleave(*[inv(4 * t + i) for i in range(4)]))

    with jax.named_scope("out"):
        cp_o = [pltpu.make_async_copy(xb.at[c], out_hbm.at[:, col(c)], sems.at[8 + c])
                for c in range(8)]
        bits = lambda v: lax.bitcast_convert_type(v.astype(BF16).astype(F32), jnp.int32)
        for c in range(8):
            for j in range(NS // 2):
                w = (lax.shift_right_logical(bits(xt[2 * j, col(c), :]), 16)
                     | bits(xt[2 * j + 1, col(c), :]))
                xw[c, pl.ds(j, L, stride=NS // 2), :] = w.T
            cp_o[c].start()
        for d in cp_o:
            d.wait()


@jax.jit
def pallas_interleave_layers__sliding_local_dilated__spectral_gfnet__prompt_kernel(
        A_x, A_wqkv, A_wo, B_x, B_w_r, B_w_i):
    del B_x
    hbm = pl.BlockSpec(memory_space=pltpu.HBM)
    vmem = pl.BlockSpec(memory_space=pltpu.VMEM)
    out = pl.pallas_call(
        _kernel,
        out_shape=jax.ShapeDtypeStruct((S, D), BF16),
        in_specs=[hbm] * 6 + [vmem] * 6,
        out_specs=hbm,
        scratch_shapes=[
            pltpu.VMEM((NS, D, L), F32),
            pltpu.VMEM((8, S, L), BF16),
            pltpu.VMEM((4, D, D), BF16),
            pltpu.VMEM((2 * D, D), jnp.int32),
            pltpu.VMEM((2, D // 2 + 1, S), BF16),
            pltpu.VMEM((4, 512, L), F32),
            pltpu.VMEM((2 * NS, FR, L), F32),
            pltpu.VMEM((NS, 3, L, L), BF16),
            pltpu.VMEM((NS, D, L), BF16),
            pltpu.VMEM((D, L), F32),
            pltpu.VMEM((D, L), BF16),
            pltpu.VMEM((2 * NS, 2 * D, L), F32),
            pltpu.VMEM((NS, D, L), BF16),
            pltpu.VMEM((NS, 2, FR, L), F32),
            pltpu.VMEM((NS, 3, FR, L), BF16),
            pltpu.SemaphoreType.DMA((16,)),
        ],
        compiler_params=pltpu.CompilerParams(vmem_limit_bytes=124 * 1024 * 1024),
    )(A_x.reshape(S, D), A_wqkv, A_wo, B_w_r.T, B_w_i.T, *_CONSTS)
    return out.reshape(1, S, D)
```
